```python
import jax
import jax.numpy as jnp

def _softmax(x, axis=-1):
    return jax.nn.softmax(x, axis=axis)
def _gelu(x):
    return jax.nn.gelu(x, approximate=True)
def _silu(x):
    return jax.nn.silu(x)
def _sigmoid(x):
    return jax.nn.sigmoid(x)
def _layernorm(x, axis=-1, eps=1e-5):
    m = jnp.mean(x, axis=axis, keepdims=True)
    v = jnp.var(x, axis=axis, keepdims=True)
    return (x - m) / jnp.sqrt(v + eps)
def _scatter_add(tgt, idx, src, axis=0):
    return tgt.at[idx].add(src)
def _segment_sum(src, seg, n):
    return jax.ops.segment_sum(src, seg, n)
class _Rng:
    def __init__(self, key):
        self._k = key
    def _next(self):
        self._k, sub = jax.random.split(self._k)
        return sub
    def normal(self, shape):
        return jax.random.normal(self._next(), shape, dtype=jnp.bfloat16)
    def randint(self, lo, hi, shape):
        return jax.random.randint(self._next(), shape, lo, hi, dtype=jnp.int32)
    def uniform(self, shape, lo=0.0, hi=1.0):
        return jax.random.uniform(self._next(), shape, jnp.bfloat16, lo, hi)
    def permutation(self, n):
        return jax.random.permutation(self._next(), n)


kernel_name = 'gated_mix__compressed_kv_cla__sliding_local_dilated__prompt'

def setup_inputs():
    _rng = _Rng(jax.random.key(int.from_bytes(__import__("os").urandom(4), "little")))
    _w = (lambda a: (lambda t: t.astype(jnp.bfloat16) if jnp.issubdtype(t.dtype, jnp.floating) else t)(jnp.asarray(a)))
    def _A_setup():
        B, H, Sq, Sk, D, M = 1, 32, 2048, 2048, 128, 1024
        Dc = 4 * D
        return {
            "x": _w((lambda *s: _rng.normal(s) * 0.05)(B, Sq, M)),
            "c_kv": _w((lambda *s: _rng.normal(s) * 0.05)(B, Sk, Dc)),
            "w_q": _w((lambda *s: _rng.normal(s) * 0.05)(M, H, D) * (M ** -0.5)),
            "w_uk": _w((lambda *s: _rng.normal(s) * 0.05)(Dc, H, D) * (Dc ** -0.5)),
            "w_uv": _w((lambda *s: _rng.normal(s) * 0.05)(Dc, H, D) * (Dc ** -0.5)),
            "w_o": _w((lambda *s: _rng.normal(s) * 0.05)(H, D, M) * ((H * D) ** -0.5)),
        }
    _A_in = _A_setup()

    def _B_setup():
        B, S, D = 1, 2048, 1024
        return {
            "x": _w((lambda *s: _rng.normal(s) * 0.05)(B, S, D)),
            "wqkv": _w((lambda *s: _rng.normal(s) * 0.05)(D, 3 * D)),
            "wo": _w((lambda *s: _rng.normal(s) * 0.05)(D, D)),
        }
    _B_in = _B_setup()

    return {
        "A_x": _A_in["x"],
        "A_c_kv": _A_in["c_kv"],
        "A_w_q": _A_in["w_q"],
        "A_w_uk": _A_in["w_uk"],
        "A_w_uv": _A_in["w_uv"],
        "A_w_o": _A_in["w_o"],
        "B_x": _B_in["x"],
        "B_wqkv": _B_in["wqkv"],
        "B_wo": _B_in["wo"],
        "gate_w": _w((lambda *s: _rng.normal(s) * 0.05)(1024)),
    }

def reference(A_x, A_c_kv, A_w_q, A_w_uk, A_w_uv, A_w_o, B_x, B_wqkv, B_wo, gate_w):
    def _A_ref(x, c_kv, w_q, w_uk, w_uv, w_o):
        B, Sq, M = x.shape[0], x.shape[1], x.shape[2]
        Sk = c_kv.shape[1]
        H, D = w_q.shape[1], w_q.shape[2]
        q = jnp.einsum("bqm,mhd->bhqd", x, w_q)
        k = jnp.einsum("bkc,chd->bhkd", c_kv, w_uk)
        v = jnp.einsum("bkc,chd->bhkd", c_kv, w_uv)
        scores = jnp.einsum("bhqd,bhkd->bhqk", q, k) * (D ** -0.5)
        off = Sk - Sq
        qi = jnp.arange(Sq)[:, None]
        kj = jnp.arange(Sk)[None, :]
        cmask = kj <= (qi + off)
        scores = jnp.where(cmask[None, None], scores, -1e9)
        p = _softmax(scores, axis=-1)
        ctx = jnp.einsum("bhqk,bhkd->bhqd", p, v)
        return jnp.einsum("bhqd,hdm->bqm", ctx, w_o)

    def _B_ref(x, wqkv, wo):
        B, S, D = x.shape
        H = 32; Dh = D // H
        W, dil = 8, 2
        qkv = (lambda x, *d: x.transpose(*d))((x @ wqkv).reshape(B, S, 3, H, Dh), 2, 0, 3, 1, 4)
        q, k, v = qkv[0], qkv[1], qkv[2]
        scale = Dh ** -0.5
        pos = jnp.arange(S)
        off = jnp.arange(W) * dil
        idx = pos[:, None] - off[None, :]
        mask = idx >= 0
        idx_c = jnp.where(mask, idx, 0).reshape(-1)
        kg = k[:, :, idx_c, :].reshape(B, H, S, W, Dh)
        vg = v[:, :, idx_c, :].reshape(B, H, S, W, Dh)
        logits = jnp.einsum("bhsd,bhswd->bhsw", q, kg) * scale
        logits = jnp.where(mask[None, None, :, :], logits, -1e9)
        attn = _softmax(logits, axis=-1)
        o = jnp.einsum("bhsw,bhswd->bhsd", attn, vg)
        return (lambda x, *d: x.transpose(*d))(o, 0, 2, 1, 3).reshape(B, S, D) @ wo

    x = A_x
    g = _sigmoid((x * gate_w).sum(-1, keepdims=True))
    a = _A_ref(x, A_c_kv, A_w_q, A_w_uk, A_w_uv, A_w_o)
    b = _B_ref(x, B_wqkv, B_wo)
    return g * a + (1 - g) * b
```

```python
import functools
import numpy as np
import jax
import jax.numpy as jnp
from jax import lax
import jax.experimental.pallas as pl
import jax.experimental.pallas.tpu as pltpu

CFG = dict(bq=256, rb=256)

LOG2E = 1.4426950408889634
NT = (((1,), (1,)), ((), ()))
NN = (((1,), (0,)), ((), ()))


def _dot(a, b, dims=NN):
    return lax.dot_general(a, b, dims, preferred_element_type=jnp.float32)


def _kernel(x_ref, c_ref, wq_ref, wuk_ref, wuv_ref, wo_ref, bq_ref, bk_ref, bv_ref, bo_ref, gw_ref,
            out_ref, acc_ref, g_ref, q_s, k_s, v_s, kp_s, vp_s, *, S, H, D, NB, DH, W, DIL):
    step = pl.program_id(0)
    bq = CFG["bq"]
    f32, bf16 = jnp.float32, jnp.bfloat16
    NEG = -1e9 * LOG2E

    @pl.when(step == 0)
    def _init():
        gw = gw_ref[...].astype(f32)
        M = gw.shape[1]
        for r in range(0, S, 256):
            t = None
            for j in range(0, M, 128):
                p = x_ref[r:r + 256, j:j + 128].astype(f32) * gw[:, j:j + 128]
                t = p if t is None else t + p
            z = jnp.sum(t, axis=1, keepdims=True)
            g_ref[r:r + 256, :] = jnp.broadcast_to(jax.nn.sigmoid(z), (256, 128))
        acc_ref[...] = jnp.zeros_like(acc_ref)
        pad = W * DIL
        kp_s[0:pad, :] = jnp.zeros((pad, 128), f32)
        vp_s[0:pad, :] = jnp.zeros((pad, 128), f32)

    @pl.when(step < H)
    def _a_head():
        x = x_ref[...]
        c = c_ref[...]
        q_s[...] = (_dot(x, wq_ref[...]) * (D ** -0.5 * LOG2E)).astype(bf16)
        k_s[...] = _dot(c, wuk_ref[...]).astype(bf16)
        v_s[...] = _dot(c, wuv_ref[...]).astype(bf16)
        wo = wo_ref[0]
        row = lax.broadcasted_iota(jnp.int32, (bq, bq), 0)
        col = lax.broadcasted_iota(jnp.int32, (bq, bq), 1)
        cmask = col <= row
        for i in range(S // bq):
            r0, L = i * bq, (i + 1) * bq
            q = q_s[r0:L, :]
            sd = jnp.where(cmask, _dot(q, k_s[r0:L, :], NT), NEG)
            m = jnp.max(sd, axis=1, keepdims=True)
            if i > 0:
                s = _dot(q, k_s[0:r0, :], NT)
                m = jnp.maximum(m, jnp.max(s, axis=1, keepdims=True))
            p = jnp.exp2(sd - m)
            l = jnp.sum(p, axis=1, keepdims=True)
            o = _dot(p.astype(bf16), v_s[r0:L, :])
            if i > 0:
                p = jnp.exp2(s - m)
                l = l + jnp.sum(p, axis=1, keepdims=True)
                o = o + _dot(p.astype(bf16), v_s[0:r0, :])
            ctx = (o * (g_ref[r0:L, :] / l)).astype(bf16)
            acc_ref[r0:L, :] += _dot(ctx, wo)

    @pl.when(step >= H)
    def _b_tile():
        x = x_ref[...]
        pad = W * DIL
        rb = CFG["rb"]
        qf = _dot(x, bq_ref[...])
        kp_s[pad:pad + S, :] = _dot(x, bk_ref[...])
        vp_s[pad:pad + S, :] = _dot(x, bv_ref[...])
        q_s[...] = qf.astype(bf16)
        ri = lax.broadcasted_iota(jnp.int32, (128, 128), 0)
        ci = lax.broadcasted_iota(jnp.int32, (128, 128), 1)
        E = jnp.where(ri // DH == ci // DH, 1.0, 0.0).astype(bf16)
        wo = bo_ref[...]
        sc = DH ** -0.5 * LOG2E
        for r0 in range(0, S, rb):
            q = q_s[r0:r0 + rb, :].astype(f32) * sc
            lg = []
            for w in range(W):
                st = pad + r0 - w * DIL
                kw = kp_s[st:st + rb, :]
                l_w = _dot((q * kw).astype(bf16), E)
                if r0 < w * DIL:
                    rows = lax.broadcasted_iota(jnp.int32, (rb, 128), 0) + r0
                    l_w = jnp.where(rows >= w * DIL, l_w, NEG)
                lg.append(l_w)
            m = functools.reduce(jnp.maximum, lg)
            o = None
            den = None
            for w in range(W):
                st = pad + r0 - w * DIL
                p = jnp.exp2(lg[w] - m)
                pv = p * vp_s[st:st + rb, :]
                o = pv if o is None else o + pv
                den = p if den is None else den + p
            ctx = (o * ((1.0 - g_ref[r0:r0 + rb, :]) / den)).astype(bf16)
            acc_ref[r0:r0 + rb, :] += _dot(ctx, wo)

    @pl.when(step == H + NB - 1)
    def _fin():
        out_ref[...] = acc_ref[...].astype(out_ref.dtype)


@jax.jit
def pallas_gated_mix__compressed_kv_cla__sliding_local_dilated__prompt_kernel(
A_x: jax.Array,
    A_c_kv: jax.Array,
    A_w_q: jax.Array,
    A_w_uk: jax.Array,
    A_w_uv: jax.Array,
    A_w_o: jax.Array,
    B_x: jax.Array,
    B_wqkv: jax.Array,
    B_wo: jax.Array,
    gate_w: jax.Array,
):
    del B_x
    _, S, M = A_x.shape
    Dc = A_c_kv.shape[2]
    _, H, D = A_w_q.shape
    NB = M // 128
    x = A_x.reshape(S, M)
    c = A_c_kv.reshape(S, Dc)
    wq = A_w_q.reshape(M, H * D)
    wuk = A_w_uk.reshape(Dc, H * D)
    wuv = A_w_uv.reshape(Dc, H * D)
    gw = gate_w.reshape(1, M)

    def ha(s):
        return jnp.minimum(s, H - 1)

    def hb(s):
        return jnp.maximum(s - H, 0)

    const = lambda s: (0, 0)
    in_specs = [
        pl.BlockSpec((S, M), const),
        pl.BlockSpec((S, Dc), const),
        pl.BlockSpec((M, D), lambda s: (0, ha(s))),
        pl.BlockSpec((Dc, D), lambda s: (0, ha(s))),
        pl.BlockSpec((Dc, D), lambda s: (0, ha(s))),
        pl.BlockSpec((1, D, M), lambda s: (ha(s), 0, 0)),
        pl.BlockSpec((M, 128), lambda s: (0, hb(s))),
        pl.BlockSpec((M, 128), lambda s: (0, NB + hb(s))),
        pl.BlockSpec((M, 128), lambda s: (0, 2 * NB + hb(s))),
        pl.BlockSpec((128, M), lambda s: (hb(s), 0)),
        pl.BlockSpec((1, M), const),
    ]
    kern = functools.partial(_kernel, S=S, H=H, D=D, NB=NB, DH=32, W=8, DIL=2)
    out = pl.pallas_call(
        kern,
        grid=(H + NB,),
        in_specs=in_specs,
        out_specs=pl.BlockSpec((S, M), const),
        out_shape=jax.ShapeDtypeStruct((S, M), A_x.dtype),
        scratch_shapes=[
            pltpu.VMEM((S, M), jnp.float32),
            pltpu.VMEM((S, 128), jnp.float32),
            pltpu.VMEM((S, 128), jnp.bfloat16),
            pltpu.VMEM((S, 128), jnp.bfloat16),
            pltpu.VMEM((S, 128), jnp.bfloat16),
            pltpu.VMEM((S + 16, 128), jnp.float32),
            pltpu.VMEM((S + 16, 128), jnp.float32),
        ],
        compiler_params=pltpu.CompilerParams(
            dimension_semantics=("arbitrary",),
            vmem_limit_bytes=100 * 1024 * 1024,
        ),
    )(x, c, wq, wuk, wuv, A_w_o, B_wqkv, B_wqkv, B_wqkv, B_wo, gw)
    return out.reshape(1, S, M)
```

```python
import functools
import jax
import jax.numpy as jnp
from jax import lax
import jax.experimental.pallas as pl
import jax.experimental.pallas.tpu as pltpu

CFG = dict(bq=256, rb=256, rs=32, seg="xlu")

LOG2E = 1.4426950408889634
NT = (((1,), (1,)), ((), ()))
NN = (((1,), (0,)), ((), ()))
LANES = 128
f32, bf16 = jnp.float32, jnp.bfloat16


def _dot(a, b, dims=NN):
    return lax.dot_general(a, b, dims, preferred_element_type=jnp.float32)


def _kernel(x_hbm, c_hbm, wq_hbm, wuk_hbm, wuv_hbm, wo_hbm, bw_hbm, bwo_hbm, gw_hbm,
            out_hbm,
            x_v, c_v, wq_raw, wuk_raw, wuv_raw, wq_v, wuk_v, wuv_v, wo_v, bw_raw, bwt_v, bw_v, bwo_raw, bwo_v, gw_v,
            acc_v, out_v, g_v, q_s, k_s, v_s, bq_s, bk_s, bv_s, bp_s, sems,
            *, S, M, H, D, HB, DH, W, DIL):
    NEG = -1e9 * LOG2E
    NJ = M // LANES
    PAD = W * DIL

    def cp(src, dst, i):
        return pltpu.make_async_copy(src, dst, sems.at[i])

    copies = dict(
        gw=cp(gw_hbm, gw_v, 0), x=cp(x_hbm, x_v, 1), bw=cp(bw_hbm, bw_raw, 2), bwo=cp(bwo_hbm, bwo_raw, 3),
        wuk=cp(wuk_hbm, wuk_raw, 4), wuv=cp(wuv_hbm, wuv_raw, 5), wq=cp(wq_hbm, wq_raw, 6),
        c=cp(c_hbm, c_v, 7), wo=cp(wo_hbm, wo_v, 8),
    )
    for k in ("bw", "gw", "x", "bwo", "wuk", "wuv", "wq", "c", "wo"):
        copies[k].start()

    with jax.named_scope("b_perm"):
        copies["bw"].wait()
        for n0 in range(0, 3 * M, LANES):
            wt = bw_raw[:, n0:n0 + LANES].astype(f32).T.astype(bf16)
            bwt_v[n0 // DH:n0 // DH + LANES // DH] = wt.reshape(LANES // DH, DH, M)
        for t in range(3):
            w3 = jnp.swapaxes(bwt_v[t * HB:(t + 1) * HB], 0, 1)
            bw_v[t * M:(t + 1) * M, :] = w3.reshape(M, M)
        copies["bwo"].wait()
        for m0 in range(0, M, 256):
            w3 = jnp.swapaxes(bwo_raw[:, :, m0:m0 + 256], 0, 1)
            bwo_v[:, m0:m0 + 256] = w3.reshape(M, 256)
        bk_s[0:PAD, :] = jnp.zeros((PAD, M), f32)
        bv_s[0:PAD, :] = jnp.zeros((PAD, M), f32)
        copies["gw"].wait()
        copies["x"].wait()

    RB, RS = CFG["rb"], CFG["rs"]
    sc_b = DH ** -0.5 * LOG2E

    def b_chunk(ci, carry):
        r0 = pl.multiple_of(ci * RB, RB)
        xr = x_v[pl.ds(r0, RB), :]
        gw = gw_v[...].astype(f32)
        t = None
        for j in range(NJ):
            p = xr[:, j * LANES:(j + 1) * LANES].astype(f32) * gw[:, j * LANES:(j + 1) * LANES]
            t = p if t is None else t + p
        g = jnp.broadcast_to(jax.nn.sigmoid(jnp.sum(t, axis=1, keepdims=True)), (RB, LANES))
        g_v[pl.ds(r0, RB), :] = g
        bq_s[...] = _dot(xr, bw_v[0:M, :], NT) * sc_b
        bk_s[PAD:PAD + RB, :] = _dot(xr, bw_v[M:2 * M, :], NT)
        bv_s[PAD:PAD + RB, :] = _dot(xr, bw_v[2 * M:3 * M, :], NT)
        if CFG["seg"] == "mxu":
            ri = lax.broadcasted_iota(jnp.int32, (LANES, LANES), 0)
            cj = lax.broadcasted_iota(jnp.int32, (LANES, LANES), 1)
            E = jnp.where(ri % HB == cj % HB, 1.0, 0.0).astype(bf16)
        for s0 in range(0, RB, RS):
            lg = [None] * W
            for j in range(NJ):
                q = bq_s[s0:s0 + RS, j * LANES:(j + 1) * LANES]
                for w in range(W):
                    st = PAD + s0 - w * DIL
                    p = q * bk_s[st:st + RS, j * LANES:(j + 1) * LANES]
                    lg[w] = p if lg[w] is None else lg[w] + p
            for w in range(W):
                l = lg[w]
                if CFG["seg"] == "mxu":
                    hi = l.astype(bf16)
                    lo = (l - hi.astype(f32)).astype(bf16)
                    l = _dot(hi, E) + _dot(lo, E)
                else:
                    sh = LANES // 2
                    while sh >= HB:
                        l = l + pltpu.roll(l, sh, 1)
                        sh //= 2
                if s0 < w * DIL:
                    rows = lax.broadcasted_iota(jnp.int32, (RS, LANES), 0) + (s0 + r0)
                    l = jnp.where(rows >= w * DIL, l, NEG)
                lg[w] = l
            m = functools.reduce(jnp.maximum, lg)
            ps = [jnp.exp2(l - m) for l in lg]
            den = functools.reduce(lambda a, b: a + b, ps)
            inv = (1.0 - g[s0:s0 + RS, :]) / den
            for w in range(W):
                bp_s[w, s0:s0 + RS, :] = ps[w] * inv
        out = None
        for j in range(NJ):
            o = None
            for w in range(W):
                st = PAD - w * DIL
                pv = bp_s[w] * bv_s[st:st + RB, j * LANES:(j + 1) * LANES]
                o = pv if o is None else o + pv
            d = _dot(o.astype(bf16), bwo_v[j * LANES:(j + 1) * LANES, :])
            out = d if out is None else out + d
        acc_v[pl.ds(r0, RB), :] = out
        bk_s[0:PAD, :] = bk_s[RB:RB + PAD, :]
        bv_s[0:PAD, :] = bv_s[RB:RB + PAD, :]
        return carry

    with jax.named_scope("b_main"):
        lax.fori_loop(0, S // RB, b_chunk, 0)

    def relayout(raw, dst, rows):
        def body(i, carry):
            m0 = pl.multiple_of(i * LANES, LANES)
            for h0 in range(0, H, 16):
                dst[h0:h0 + 16, pl.ds(m0, LANES), :] = jnp.swapaxes(raw[pl.ds(m0, LANES), h0:h0 + 16, :], 0, 1)
            return carry
        lax.fori_loop(0, rows // LANES, body, 0)

    with jax.named_scope("a_relayout"):
        copies["wuk"].wait()
        relayout(wuk_raw, wuk_v, wuk_raw.shape[0])
        copies["wuv"].wait()
        relayout(wuv_raw, wuv_v, wuv_raw.shape[0])
        copies["wq"].wait()
        relayout(wq_raw, wq_v, wq_raw.shape[0])
        copies["c"].wait()
        copies["wo"].wait()

    BQ = CFG["bq"]
    sc_a = D ** -0.5 * LOG2E

    def a_head(h, carry):
        x = x_v[...]
        c = c_v[...]
        q_s[...] = (_dot(x, wq_v[h]) * sc_a).astype(bf16)
        k_s[...] = _dot(c, wuk_v[h]).astype(bf16)
        v_s[...] = _dot(c, wuv_v[h]).astype(bf16)
        wo = wo_v[h]
        row = lax.broadcasted_iota(jnp.int32, (LANES, LANES), 0)
        col = lax.broadcasted_iota(jnp.int32, (LANES, LANES), 1)
        cmask = col <= row
        for i in range(S // BQ):
            r0 = i * BQ
            q = q_s[r0:r0 + BQ, :]
            if i > 0:
                s = _dot(q, k_s[0:r0, :], NT)
                m_off = jnp.max(s, axis=1, keepdims=True)
            sd, md = [], []
            for a in range(BQ // LANES):
                qa = q[a * LANES:(a + 1) * LANES]
                t = _dot(qa, k_s[r0:r0 + (a + 1) * LANES, :], NT)
                tiles = [t[:, b * LANES:(b + 1) * LANES] for b in range(a + 1)]
                tiles[a] = jnp.where(cmask, tiles[a], NEG)
                t = jnp.concatenate(tiles, axis=1) if a > 0 else tiles[0]
                m = jnp.max(t, axis=1, keepdims=True)
                if i > 0:
                    m = jnp.maximum(m, m_off[a * LANES:(a + 1) * LANES])
                sd.append(t)
                md.append(m)
            m = jnp.concatenate(md, axis=0)
            if i > 0:
                p = jnp.exp2(s - m)
                l_off = jnp.sum(p, axis=1, keepdims=True)
                o_off = _dot(p.astype(bf16), v_s[0:r0, :])
            ctx = []
            for a in range(BQ // LANES):
                p = jnp.exp2(sd[a] - md[a])
                l = jnp.sum(p, axis=1, keepdims=True)
                o = _dot(p.astype(bf16), v_s[r0:r0 + (a + 1) * LANES, :])
                if i > 0:
                    l = l + l_off[a * LANES:(a + 1) * LANES]
                    o = o + o_off[a * LANES:(a + 1) * LANES]
                ctx.append((o * (g_v[r0 + a * LANES:r0 + (a + 1) * LANES, :] / l)).astype(bf16))
            ctx = jnp.concatenate(ctx, axis=0)
            acc_v[r0:r0 + BQ, :] += _dot(ctx, wo)
        return carry

    with jax.named_scope("a_main"):
        lax.fori_loop(0, H, a_head, 0)

    with jax.named_scope("final"):
        out_v[...] = acc_v[...].astype(out_v.dtype)
        oc = cp(out_v, out_hbm, 9)
        oc.start()
        oc.wait()


@jax.jit
def pallas_gated_mix__compressed_kv_cla__sliding_local_dilated__prompt_kernel(
A_x: jax.Array,
    A_c_kv: jax.Array,
    A_w_q: jax.Array,
    A_w_uk: jax.Array,
    A_w_uv: jax.Array,
    A_w_o: jax.Array,
    B_x: jax.Array,
    B_wqkv: jax.Array,
    B_wo: jax.Array,
    gate_w: jax.Array,
):
    del B_x
    _, S, M = A_x.shape
    Dc = A_c_kv.shape[2]
    _, H, D = A_w_q.shape
    HB, W, DIL = 32, 8, 2
    DH = M // HB
    PAD = W * DIL
    RB = CFG["rb"]
    dt = A_x.dtype
    hbm = pl.BlockSpec(memory_space=pltpu.MemorySpace.HBM)
    V = pltpu.VMEM
    kern = functools.partial(_kernel, S=S, M=M, H=H, D=D, HB=HB, DH=DH, W=W, DIL=DIL)
    out = pl.pallas_call(
        kern,
        in_specs=[hbm] * 9,
        out_specs=hbm,
        out_shape=jax.ShapeDtypeStruct((S, M), dt),
        scratch_shapes=[
            V((S, M), dt), V((S, Dc), dt),
            V((M, H, D), dt), V((Dc, H, D), dt), V((Dc, H, D), dt),
            V((H, M, D), dt), V((H, Dc, D), dt), V((H, Dc, D), dt), V((H, D, M), dt),
            V((M, 3 * M), dt), V((3 * HB, DH, M), dt), V((3 * M, M), dt),
            V((HB, DH, M), dt), V((M, M), dt), V((1, M), dt),
            V((S, M), f32), V((S, M), dt), V((S, LANES), f32),
            V((S, D), dt), V((S, D), dt), V((S, D), dt),
            V((RB, M), f32), V((RB + PAD, M), f32), V((RB + PAD, M), f32), V((W, RB, LANES), f32),
            pltpu.SemaphoreType.DMA((10,)),
        ],
        compiler_params=pltpu.CompilerParams(vmem_limit_bytes=110 * 1024 * 1024),
    )(A_x.reshape(S, M), A_c_kv.reshape(S, Dc), A_w_q, A_w_uk, A_w_uv, A_w_o,
      B_wqkv, B_wo.reshape(HB, DH, M), gate_w.reshape(1, M))
    return out.reshape(1, S, M)
```

```python
import functools
import jax
import jax.numpy as jnp
from jax import lax
import jax.experimental.pallas as pl
import jax.experimental.pallas.tpu as pltpu

CFG = dict(bq=256, ck=512, cn=512, rb=256, rs=32, seg="xlu")

LOG2E = 1.4426950408889634
NT = (((1,), (1,)), ((), ()))
NN = (((1,), (0,)), ((), ()))
LANES = 128
f32, bf16 = jnp.float32, jnp.bfloat16


def _dot(a, b, dims=NN):
    return lax.dot_general(a, b, dims, preferred_element_type=jnp.float32)


def _kernel(x_hbm, c_hbm, wq_hbm, wuk_hbm, wuv_hbm, wo_hbm, bw_hbm, bwo_hbm, gw_hbm,
            out_hbm,
            x_v, c_v, wq_raw, wuk_raw, wuv_raw, wq_v, wuk_v, wuv_v, wo_v, bw_raw, bwt_v, bw_v, bwo_raw, bwo_v, gw_v,
            acc_v, out_v, g_v, q_s, k_s, v_s, s_s, bq_s, bk_s, bv_s, bp_s, sems,
            *, S, M, H, D, HB, DH, W, DIL):
    NEG = -1e9 * LOG2E
    NJ = M // LANES
    PAD = W * DIL

    def cp(src, dst, i):
        return pltpu.make_async_copy(src, dst, sems.at[i])

    copies = dict(
        gw=cp(gw_hbm, gw_v, 0), x=cp(x_hbm, x_v, 1), bw=cp(bw_hbm, bw_raw, 2), bwo=cp(bwo_hbm, bwo_raw, 3),
        wuk=cp(wuk_hbm, wuk_raw, 4), wuv=cp(wuv_hbm, wuv_raw, 5), wq=cp(wq_hbm, wq_raw, 6),
        c=cp(c_hbm, c_v, 7), wo=cp(wo_hbm, wo_v, 8),
    )
    for k in ("bw", "gw", "x", "bwo", "wuk", "wuv", "wq", "c", "wo"):
        copies[k].start()

    with jax.named_scope("b_perm"):
        copies["bw"].wait()
        for n0 in range(0, 3 * M, LANES):
            wt = bw_raw[:, n0:n0 + LANES].astype(f32).T.astype(bf16)
            bwt_v[n0 // DH:n0 // DH + LANES // DH] = wt.reshape(LANES // DH, DH, M)
        for t in range(3):
            w3 = jnp.swapaxes(bwt_v[t * HB:(t + 1) * HB], 0, 1)
            bw_v[t * M:(t + 1) * M, :] = w3.reshape(M, M)
        copies["bwo"].wait()
        for m0 in range(0, M, 256):
            w3 = jnp.swapaxes(bwo_raw[:, :, m0:m0 + 256], 0, 1)
            bwo_v[:, m0:m0 + 256] = w3.reshape(M, 256)
        bk_s[0:PAD, :] = jnp.zeros((PAD, M), f32)
        bv_s[0:PAD, :] = jnp.zeros((PAD, M), f32)
        copies["gw"].wait()
        copies["x"].wait()

    RB, RS = CFG["rb"], CFG["rs"]
    sc_b = DH ** -0.5 * LOG2E

    def b_chunk(ci, carry):
        r0 = pl.multiple_of(ci * RB, RB)
        xr = x_v[pl.ds(r0, RB), :]
        gw = gw_v[...].astype(f32)
        t = None
        for j in range(NJ):
            p = xr[:, j * LANES:(j + 1) * LANES].astype(f32) * gw[:, j * LANES:(j + 1) * LANES]
            t = p if t is None else t + p
        g = jnp.broadcast_to(jax.nn.sigmoid(jnp.sum(t, axis=1, keepdims=True)), (RB, LANES))
        g_v[pl.ds(r0, RB), :] = g
        bq_s[...] = _dot(xr, bw_v[0:M, :], NT) * sc_b
        bk_s[PAD:PAD + RB, :] = _dot(xr, bw_v[M:2 * M, :], NT)
        bv_s[PAD:PAD + RB, :] = _dot(xr, bw_v[2 * M:3 * M, :], NT)
        if CFG["seg"] == "mxu":
            ri = lax.broadcasted_iota(jnp.int32, (LANES, LANES), 0)
            cj = lax.broadcasted_iota(jnp.int32, (LANES, LANES), 1)
            E = jnp.where(ri % HB == cj % HB, 1.0, 0.0).astype(bf16)
        for s0 in range(0, RB, RS):
            lg = [None] * W
            for j in range(NJ):
                q = bq_s[s0:s0 + RS, j * LANES:(j + 1) * LANES]
                for w in range(W):
                    st = PAD + s0 - w * DIL
                    p = q * bk_s[st:st + RS, j * LANES:(j + 1) * LANES]
                    lg[w] = p if lg[w] is None else lg[w] + p
            for w in range(W):
                l = lg[w]
                if CFG["seg"] == "mxu":
                    hi = l.astype(bf16)
                    lo = (l - hi.astype(f32)).astype(bf16)
                    l = _dot(hi, E) + _dot(lo, E)
                else:
                    sh = LANES // 2
                    while sh >= HB:
                        l = l + pltpu.roll(l, sh, 1)
                        sh //= 2
                if s0 < w * DIL:
                    rows = lax.broadcasted_iota(jnp.int32, (RS, LANES), 0) + (s0 + r0)
                    l = jnp.where(rows >= w * DIL, l, NEG)
                lg[w] = l
            m = functools.reduce(jnp.maximum, lg)
            ps = [jnp.exp2(l - m) for l in lg]
            den = functools.reduce(lambda a, b: a + b, ps)
            inv = (1.0 - g[s0:s0 + RS, :]) / den
            for w in range(W):
                bp_s[w, s0:s0 + RS, :] = ps[w] * inv
        out = None
        for j in range(NJ):
            o = None
            for w in range(W):
                st = PAD - w * DIL
                pv = bp_s[w] * bv_s[st:st + RB, j * LANES:(j + 1) * LANES]
                o = pv if o is None else o + pv
            d = _dot(o.astype(bf16), bwo_v[j * LANES:(j + 1) * LANES, :])
            out = d if out is None else out + d
        acc_v[pl.ds(r0, RB), :] = out
        bk_s[0:PAD, :] = bk_s[RB:RB + PAD, :]
        bv_s[0:PAD, :] = bv_s[RB:RB + PAD, :]
        return carry

    with jax.named_scope("b_main"):
        lax.fori_loop(0, S // RB, b_chunk, 0)

    def relayout(raw, dst, rows):
        def body(i, carry):
            m0 = pl.multiple_of(i * LANES, LANES)
            for h0 in range(0, H, 16):
                dst[h0:h0 + 16, pl.ds(m0, LANES), :] = jnp.swapaxes(raw[pl.ds(m0, LANES), h0:h0 + 16, :], 0, 1)
            return carry
        lax.fori_loop(0, rows // LANES, body, 0)

    with jax.named_scope("a_relayout"):
        copies["wuk"].wait()
        relayout(wuk_raw, wuk_v, wuk_raw.shape[0])
        copies["wuv"].wait()
        relayout(wuv_raw, wuv_v, wuv_raw.shape[0])
        copies["wq"].wait()
        relayout(wq_raw, wq_v, wq_raw.shape[0])
        copies["c"].wait()
        copies["wo"].wait()

    BQ, CK, CN = CFG["bq"], CFG["ck"], CFG["cn"]
    T = LANES
    NA = BQ // T
    sc_a = D ** -0.5 * LOG2E

    def pieces(i):
        r0 = i * BQ
        ps = [(0, k0, min(k0 + CK, r0), False) for k0 in range(0, r0, CK)]
        ps += [(b, r0 + b * T, r0 + (b + 1) * T, True) for b in range(NA)]
        return ps

    def a_head(h, carry):
        x = x_v[...]
        c = c_v[...]
        q_s[...] = (_dot(x, wq_v[h]) * sc_a).astype(bf16)
        k_s[...] = _dot(c, wuk_v[h]).astype(bf16)
        v_s[...] = _dot(c, wuv_v[h]).astype(bf16)
        row = lax.broadcasted_iota(jnp.int32, (T, T), 0)
        col = lax.broadcasted_iota(jnp.int32, (T, T), 1)
        cmask = col <= row
        st = {}

        def acc(lst, a, v, op):
            lst[a] = v if lst[a] is None else op(lst[a], v)

        def qk(i, pc):
            a0, k0, k1, diag = pc
            d = st.setdefault(i, dict(mr=[None] * NA, m=[None] * NA, l=[None] * NA, o=[None] * NA))
            r0 = i * BQ
            sc = _dot(q_s[r0 + a0 * T:r0 + BQ, :], k_s[k0:k1, :], NT)
            for a in range(a0, NA):
                sa = sc[(a - a0) * T:(a - a0 + 1) * T]
                if diag and a == a0:
                    sa = jnp.where(cmask, sa, NEG)
                s_s[i % 2, a * T:(a + 1) * T, k0:k1] = sa
                acc(d["mr"], a, functools.reduce(jnp.maximum, [sa[:, t:t + T] for t in range(0, k1 - k0, T)]),
                    jnp.maximum)

        def fin_m(i):
            d = st[i]
            for a in range(NA):
                d["m"][a] = jnp.max(d["mr"][a], axis=1, keepdims=True)

        def pv(i, pc):
            a0, k0, k1, diag = pc
            d = st[i]
            ps = []
            for a in range(a0, NA):
                p = jnp.exp2(s_s[i % 2, a * T:(a + 1) * T, k0:k1] - d["m"][a])
                acc(d["l"], a, functools.reduce(lambda u, v: u + v, [p[:, t:t + T] for t in range(0, k1 - k0, T)]),
                    lambda u, v: u + v)
                ps.append(p.astype(bf16))
            o = _dot(ps[0] if len(ps) == 1 else jnp.concatenate(ps, axis=0), v_s[k0:k1, :])
            for a in range(a0, NA):
                acc(d["o"], a, o[(a - a0) * T:(a - a0 + 1) * T], lambda u, v: u + v)

        def fin_o(i):
            d = st[i]
            r0 = i * BQ
            ctx = []
            for a in range(NA):
                l = jnp.sum(d["l"][a], axis=1, keepdims=True)
                ctx.append((d["o"][a] * (g_v[r0 + a * T:r0 + (a + 1) * T, :] / l)).astype(bf16))
            d["ctx"] = ctx[0] if NA == 1 else jnp.concatenate(ctx, axis=0)

        def outp(i, n0):
            r0 = i * BQ
            acc_v[r0:r0 + BQ, n0:n0 + CN] += _dot(st[i]["ctx"], wo_v[h, :, n0:n0 + CN])

        def interleave(*streams):
            streams = [s_ for s_ in streams if s_]
            n = max(len(s_) for s_ in streams)
            pos = [0] * len(streams)
            for t in range(n):
                for j, s_ in enumerate(streams):
                    want = ((t + 1) * len(s_) + n - 1) // n
                    while pos[j] < want:
                        s_[pos[j]]()
                        pos[j] += 1

        nq = S // BQ
        for pc in pieces(0):
            qk(0, pc)
        for i in range(nq):
            fin_m(i)
            s_qk = [functools.partial(qk, i + 1, pc) for pc in pieces(i + 1)] if i + 1 < nq else []
            s_pv = [functools.partial(pv, i, pc) for pc in pieces(i)]
            s_o = [functools.partial(outp, i - 1, n0) for n0 in range(0, M, CN)] if i > 0 else []
            interleave(s_qk, s_pv, s_o)
            fin_o(i)
        for n0 in range(0, M, CN):
            outp(nq - 1, n0)
        return carry

    with jax.named_scope("a_main"):
        lax.fori_loop(0, H, a_head, 0)

    with jax.named_scope("final"):
        out_v[...] = acc_v[...].astype(out_v.dtype)
        oc = cp(out_v, out_hbm, 9)
        oc.start()
        oc.wait()


@jax.jit
def pallas_gated_mix__compressed_kv_cla__sliding_local_dilated__prompt_kernel(
A_x: jax.Array,
    A_c_kv: jax.Array,
    A_w_q: jax.Array,
    A_w_uk: jax.Array,
    A_w_uv: jax.Array,
    A_w_o: jax.Array,
    B_x: jax.Array,
    B_wqkv: jax.Array,
    B_wo: jax.Array,
    gate_w: jax.Array,
):
    del B_x
    _, S, M = A_x.shape
    Dc = A_c_kv.shape[2]
    _, H, D = A_w_q.shape
    HB, W, DIL = 32, 8, 2
    DH = M // HB
    PAD = W * DIL
    RB = CFG["rb"]
    dt = A_x.dtype
    hbm = pl.BlockSpec(memory_space=pltpu.MemorySpace.HBM)
    V = pltpu.VMEM
    kern = functools.partial(_kernel, S=S, M=M, H=H, D=D, HB=HB, DH=DH, W=W, DIL=DIL)
    out = pl.pallas_call(
        kern,
        in_specs=[hbm] * 9,
        out_specs=hbm,
        out_shape=jax.ShapeDtypeStruct((S, M), dt),
        scratch_shapes=[
            V((S, M), dt), V((S, Dc), dt),
            V((M, H, D), dt), V((Dc, H, D), dt), V((Dc, H, D), dt),
            V((H, M, D), dt), V((H, Dc, D), dt), V((H, Dc, D), dt), V((H, D, M), dt),
            V((M, 3 * M), dt), V((3 * HB, DH, M), dt), V((3 * M, M), dt),
            V((HB, DH, M), dt), V((M, M), dt), V((1, M), dt),
            V((S, M), f32), V((S, M), dt), V((S, LANES), f32),
            V((S, D), dt), V((S, D), dt), V((S, D), dt), V((2, CFG["bq"], S), f32),
            V((RB, M), f32), V((RB + PAD, M), f32), V((RB + PAD, M), f32), V((W, RB, LANES), f32),
            pltpu.SemaphoreType.DMA((10,)),
        ],
        compiler_params=pltpu.CompilerParams(vmem_limit_bytes=110 * 1024 * 1024),
    )(A_x.reshape(S, M), A_c_kv.reshape(S, Dc), A_w_q, A_w_uk, A_w_uv, A_w_o,
      B_wqkv, B_wo.reshape(HB, DH, M), gate_w.reshape(1, M))
    return out.reshape(1, S, M)
```

```python
import functools
import jax
import jax.numpy as jnp
from jax import lax
import jax.experimental.pallas as pl
import jax.experimental.pallas.tpu as pltpu

CFG = dict(rot=0, bq=128, ck=256, cn=512, pr=256, pre=1, post=2, rb=256, rs=32, seg="xlu")

LOG2E = 1.4426950408889634
NT = (((1,), (1,)), ((), ()))
NN = (((1,), (0,)), ((), ()))
LANES = 128
f32, bf16 = jnp.float32, jnp.bfloat16


def _dot(a, b, dims=NN):
    return lax.dot_general(a, b, dims, preferred_element_type=jnp.float32)


def _kernel(x_hbm, c_hbm, wq_hbm, wuk_hbm, wuv_hbm, wo_hbm, bw_hbm, bwo_hbm, gw_hbm,
            out_hbm,
            x_v, c_v, wq_raw, wuk_raw, wuv_raw, wq_v, wuk_v, wuv_v, wo_v, bw_raw, bwt_v, bw_v, bwo_raw, bwo_v, gw_v,
            acc_v, out_v, g_v, q_s, k_s, v_s, q_n, k_n, v_n, s_s, bq_s, bk_s, bv_s, bp_s, sems, osems,
            *, S, M, H, D, HB, DH, W, DIL):
    NEG = -1e9 * LOG2E
    NJ = M // LANES
    PAD = W * DIL

    def cp(src, dst, i):
        return pltpu.make_async_copy(src, dst, sems.at[i])

    copies = dict(
        gw=cp(gw_hbm, gw_v, 0), x=cp(x_hbm, x_v, 1), bw=cp(bw_hbm, bw_raw, 2), bwo=cp(bwo_hbm, bwo_raw, 3),
        wuk=cp(wuk_hbm, wuk_raw, 4), wuv=cp(wuv_hbm, wuv_raw, 5), wq=cp(wq_hbm, wq_raw, 6),
        c=cp(c_hbm, c_v, 7), wo=cp(wo_hbm, wo_v, 8),
    )
    for k in ("bw", "gw", "x", "bwo", "wuk", "wuv", "wq", "c", "wo"):
        copies[k].start()

    with jax.named_scope("b_perm"):
        copies["bw"].wait()
        for n0 in range(0, 3 * M, LANES):
            wt = bw_raw[:, n0:n0 + LANES].astype(f32).T.astype(bf16)
            bwt_v[n0 // DH:n0 // DH + LANES // DH] = wt.reshape(LANES // DH, DH, M)
        for t in range(3):
            w3 = jnp.swapaxes(bwt_v[t * HB:(t + 1) * HB], 0, 1)
            bw_v[t * M:(t + 1) * M, :] = w3.reshape(M, M)
        copies["bwo"].wait()
        for m0 in range(0, M, 256):
            w3 = jnp.swapaxes(bwo_raw[:, :, m0:m0 + 256], 0, 1)
            bwo_v[:, m0:m0 + 256] = w3.reshape(M, 256)
        bk_s[0:PAD, :] = jnp.zeros((PAD, M), f32)
        bv_s[0:PAD, :] = jnp.zeros((PAD, M), f32)
        copies["gw"].wait()
        copies["x"].wait()

    RB, RS = CFG["rb"], CFG["rs"]
    sc_b = DH ** -0.5 * LOG2E

    def b_chunk(ci, carry):
        r0 = pl.multiple_of(ci * RB, RB)
        xr = x_v[pl.ds(r0, RB), :]
        gw = gw_v[...].astype(f32)
        t = None
        for j in range(NJ):
            p = xr[:, j * LANES:(j + 1) * LANES].astype(f32) * gw[:, j * LANES:(j + 1) * LANES]
            t = p if t is None else t + p
        g = jnp.broadcast_to(jax.nn.sigmoid(jnp.sum(t, axis=1, keepdims=True)), (RB, LANES))
        g_v[pl.ds(r0, RB), :] = g
        bq_s[...] = _dot(xr, bw_v[0:M, :], NT) * sc_b
        bk_s[PAD:PAD + RB, :] = _dot(xr, bw_v[M:2 * M, :], NT)
        bv_s[PAD:PAD + RB, :] = _dot(xr, bw_v[2 * M:3 * M, :], NT)
        if CFG["seg"] == "mxu":
            ri = lax.broadcasted_iota(jnp.int32, (LANES, LANES), 0)
            cj = lax.broadcasted_iota(jnp.int32, (LANES, LANES), 1)
            E = jnp.where(ri % HB == cj % HB, 1.0, 0.0).astype(bf16)
        for s0 in range(0, RB, RS):
            lg = [None] * W
            for j in range(NJ):
                q = bq_s[s0:s0 + RS, j * LANES:(j + 1) * LANES]
                for w in range(W):
                    st = PAD + s0 - w * DIL
                    p = q * bk_s[st:st + RS, j * LANES:(j + 1) * LANES]
                    lg[w] = p if lg[w] is None else lg[w] + p
            for w in range(W):
                l = lg[w]
                if CFG["seg"] == "mxu":
                    hi = l.astype(bf16)
                    lo = (l - hi.astype(f32)).astype(bf16)
                    l = _dot(hi, E) + _dot(lo, E)
                else:
                    sh = LANES // 2
                    while sh >= HB:
                        l = l + pltpu.roll(l, sh, 1)
                        sh //= 2
                if s0 < w * DIL:
                    rows = lax.broadcasted_iota(jnp.int32, (RS, LANES), 0) + (s0 + r0)
                    l = jnp.where(rows >= w * DIL, l, NEG)
                lg[w] = l
            m = functools.reduce(jnp.maximum, lg)
            ps = [jnp.exp2(l - m) for l in lg]
            den = functools.reduce(lambda a, b: a + b, ps)
            inv = (1.0 - g[s0:s0 + RS, :]) / den
            for w in range(W):
                bp_s[w, s0:s0 + RS, :] = ps[w] * inv
        out = None
        for j in range(NJ):
            o = None
            for w in range(W):
                st = PAD - w * DIL
                pv = bp_s[w] * bv_s[st:st + RB, j * LANES:(j + 1) * LANES]
                o = pv if o is None else o + pv
            d = _dot(o.astype(bf16), bwo_v[j * LANES:(j + 1) * LANES, :])
            out = d if out is None else out + d
        acc_v[pl.ds(r0, RB), :] = out
        bk_s[0:PAD, :] = bk_s[RB:RB + PAD, :]
        bv_s[0:PAD, :] = bv_s[RB:RB + PAD, :]
        return carry

    with jax.named_scope("b_main"):
        lax.fori_loop(0, S // RB, b_chunk, 0)

    def relayout(raw, dst, rows):
        def body(i, carry):
            m0 = pl.multiple_of(i * LANES, LANES)
            for h0 in range(0, H, 16):
                dst[h0:h0 + 16, pl.ds(m0, LANES), :] = jnp.swapaxes(raw[pl.ds(m0, LANES), h0:h0 + 16, :], 0, 1)
            return carry
        lax.fori_loop(0, rows // LANES, body, 0)

    with jax.named_scope("a_relayout"):
        copies["wuk"].wait()
        relayout(wuk_raw, wuk_v, wuk_raw.shape[0])
        copies["wuv"].wait()
        relayout(wuv_raw, wuv_v, wuv_raw.shape[0])
        copies["wq"].wait()
        relayout(wq_raw, wq_v, wq_raw.shape[0])
        copies["c"].wait()
        copies["wo"].wait()

    BQ, CK, CN = CFG["bq"], CFG["ck"], CFG["cn"]
    T = LANES
    NA = BQ // T
    sc_a = D ** -0.5 * LOG2E

    def pieces(i):
        r0 = i * BQ
        ps = [(0, k0, min(k0 + CK, r0), False) for k0 in range(0, r0, CK)]
        ps += [(b, r0 + b * T, r0 + (b + 1) * T, True) for b in range(NA)]
        return ps

    PR = CFG["pr"]

    def proj_pieces(hn, qd, kd, vd):
        def pq(r):
            qd[r:r + PR, :] = (_dot(x_v[r:r + PR, :], wq_v[hn]) * sc_a).astype(bf16)
        def pk(r):
            kd[r:r + PR, :] = _dot(c_v[r:r + PR, :], wuk_v[hn]).astype(bf16)
        def pvv(r):
            vd[r:r + PR, :] = _dot(c_v[r:r + PR, :], wuv_v[hn]).astype(bf16)
        qk_, v_ = [], []
        for r in range(0, S, PR):
            qk_.append([functools.partial(pk, r), functools.partial(pq, r)])
            v_.append([functools.partial(pvv, r)])
        lag = min(CFG["post"], S // PR)
        out = []
        for n in range(len(qk_) + lag):
            if n < len(qk_):
                out += qk_[n]
            if n >= lag:
                out += v_[n - lag]
        return out

    def copy_pieces(pairs):
        def cpy(src, dst, r):
            dst[r:r + 256, :] = src[r:r + 256, :]
        return [functools.partial(cpy, a_, b_, r) for r in range(0, S, 256) for a_, b_ in pairs]

    def a_head(h, last):
        row = lax.broadcasted_iota(jnp.int32, (T, T), 0)
        col = lax.broadcasted_iota(jnp.int32, (T, T), 1)
        cmask = col <= row
        st = {}

        def acc(lst, a, v, op):
            lst[a] = v if lst[a] is None else op(lst[a], v)

        def qk(i, pc):
            a0, k0, k1, diag = pc
            d = st.setdefault(i, dict(mr=[None] * NA, m=[None] * NA, l=[None] * NA, o=[None] * NA))
            r0 = i * BQ
            sc = _dot(q_s[r0 + a0 * T:r0 + BQ, :], k_s[k0:k1, :], NT)
            for a in range(a0, NA):
                sa = sc[(a - a0) * T:(a - a0 + 1) * T]
                if diag and a == a0:
                    sa = jnp.where(cmask, sa, NEG)
                s_s[i % 2, a * T:(a + 1) * T, k0:k1] = sa
                acc(d["mr"], a, functools.reduce(jnp.maximum, [sa[:, t:t + T] for t in range(0, k1 - k0, T)]),
                    jnp.maximum)

        def fin_m(i):
            d = st[i]
            for a in range(NA):
                d["m"][a] = jnp.max(d["mr"][a], axis=1, keepdims=True)

        def pv(i, pc):
            a0, k0, k1, diag = pc
            d = st[i]
            ps = []
            for a in range(a0, NA):
                p = jnp.exp2(s_s[i % 2, a * T:(a + 1) * T, k0:k1] - d["m"][a])
                acc(d["l"], a, functools.reduce(lambda u, v: u + v, [p[:, t:t + T] for t in range(0, k1 - k0, T)]),
                    lambda u, v: u + v)
                ps.append(p.astype(bf16))
            o = _dot(ps[0] if len(ps) == 1 else jnp.concatenate(ps, axis=0), v_s[k0:k1, :])
            for a in range(a0, NA):
                acc(d["o"], a, o[(a - a0) * T:(a - a0 + 1) * T], lambda u, v: u + v)

        def fin_o(i):
            d = st[i]
            r0 = i * BQ
            ctx = []
            for a in range(NA):
                l = jnp.sum(d["l"][a], axis=1, keepdims=True)
                ctx.append((d["o"][a] * (g_v[r0 + a * T:r0 + (a + 1) * T, :] / l)).astype(bf16))
            d["ctx"] = ctx[0] if NA == 1 else jnp.concatenate(ctx, axis=0)

        def outp(i, n0):
            r0 = i * BQ
            upd = acc_v[r0:r0 + BQ, n0:n0 + CN] + _dot(st[i]["ctx"], wo_v[h, :, n0:n0 + CN])
            if not last:
                acc_v[r0:r0 + BQ, n0:n0 + CN] = upd
            else:
                out_v[r0:r0 + BQ, n0:n0 + CN] = upd.astype(out_v.dtype)
                if n0 + CN == M:
                    out_copy(i).start()

        def interleave(*streams):
            streams = [s_ for s_ in streams if s_]
            n = max(len(s_) for s_ in streams)
            pos = [0] * len(streams)
            for t in range(n):
                for j, s_ in enumerate(streams):
                    want = ((t + 1) * len(s_) + n - 1) // n
                    while pos[j] < want:
                        s_[pos[j]]()
                        pos[j] += 1

        nq = S // BQ
        rot = CFG["rot"]
        if not rot:
            for f_ in proj_pieces(h, q_s, k_s, v_s):
                f_()
        nxt = [] if (last or not rot) else proj_pieces(h + 1, q_n, k_n, v_n)
        wts = [len(pieces(i)) * 2 + 2 for i in range(nq)]
        cum, tot, lo = 0, sum(wts), 0
        head_n = CFG["pre"]
        for pc in pieces(0):
            qk(0, pc)
        for f_ in nxt[:head_n]:
            f_()
        lo = head_n
        for i in range(nq):
            fin_m(i)
            cum += wts[i]
            hi = max(lo, min(len(nxt), head_n + ((len(nxt) - head_n - CFG["post"]) * cum + tot - 1) // tot))
            s_qk = [functools.partial(qk, i + 1, pc) for pc in pieces(i + 1)] if i + 1 < nq else []
            s_pv = [functools.partial(pv, i, pc) for pc in pieces(i)]
            s_o = [functools.partial(outp, i - 1, n0) for n0 in range(0, M, CN)] if i > 0 else []
            s_c = copy_pieces([(q_n, q_s), (k_n, k_s)]) if (i == nq - 1 and not last and rot) else []
            if s_c:
                for f_ in nxt[lo:hi]:
                    f_()
                lo = hi
            interleave(s_qk, s_pv, s_o, nxt[lo:hi], s_c)
            lo = hi
            fin_o(i)
        interleave([functools.partial(outp, nq - 1, n0) for n0 in range(0, M, CN)], nxt[lo:])
        if rot and not last:
            for f_ in copy_pieces([(v_n, v_s)]):
                f_()

    nq_ = S // BQ

    def out_copy(i):
        return pltpu.make_async_copy(out_v.at[pl.ds(i * BQ, BQ), :], out_hbm.at[pl.ds(i * BQ, BQ), :], osems.at[i])

    with jax.named_scope("a_first"):
        for f_ in (proj_pieces(0, q_s, k_s, v_s) if CFG["rot"] else []):
            f_()
    with jax.named_scope("a_main"):
        lax.fori_loop(0, H - 1, lambda h, c_: (a_head(h, False), c_)[1], 0)
    with jax.named_scope("a_last"):
        a_head(H - 1, True)
        for i in range(nq_):
            out_copy(i).wait()


@jax.jit
def pallas_gated_mix__compressed_kv_cla__sliding_local_dilated__prompt_kernel(
A_x: jax.Array,
    A_c_kv: jax.Array,
    A_w_q: jax.Array,
    A_w_uk: jax.Array,
    A_w_uv: jax.Array,
    A_w_o: jax.Array,
    B_x: jax.Array,
    B_wqkv: jax.Array,
    B_wo: jax.Array,
    gate_w: jax.Array,
):
    del B_x
    _, S, M = A_x.shape
    Dc = A_c_kv.shape[2]
    _, H, D = A_w_q.shape
    HB, W, DIL = 32, 8, 2
    DH = M // HB
    PAD = W * DIL
    RB = CFG["rb"]
    dt = A_x.dtype
    hbm = pl.BlockSpec(memory_space=pltpu.MemorySpace.HBM)
    V = pltpu.VMEM
    kern = functools.partial(_kernel, S=S, M=M, H=H, D=D, HB=HB, DH=DH, W=W, DIL=DIL)
    out = pl.pallas_call(
        kern,
        in_specs=[hbm] * 9,
        out_specs=hbm,
        out_shape=jax.ShapeDtypeStruct((S, M), dt),
        scratch_shapes=[
            V((S, M), dt), V((S, Dc), dt),
            V((M, H, D), dt), V((Dc, H, D), dt), V((Dc, H, D), dt),
            V((H, M, D), dt), V((H, Dc, D), dt), V((H, Dc, D), dt), V((H, D, M), dt),
            V((M, 3 * M), dt), V((3 * HB, DH, M), dt), V((3 * M, M), dt),
            V((HB, DH, M), dt), V((M, M), dt), V((1, M), dt),
            V((S, M), f32), V((S, M), dt), V((S, LANES), f32),
            V((S, D), dt), V((S, D), dt), V((S, D), dt), V((S, D), dt), V((S, D), dt), V((S, D), dt), V((2, CFG["bq"], S), f32),
            V((RB, M), f32), V((RB + PAD, M), f32), V((RB + PAD, M), f32), V((W, RB, LANES), f32),
            pltpu.SemaphoreType.DMA((10,)), pltpu.SemaphoreType.DMA((S // CFG["bq"],)),
        ],
        compiler_params=pltpu.CompilerParams(vmem_limit_bytes=110 * 1024 * 1024),
    )(A_x.reshape(S, M), A_c_kv.reshape(S, Dc), A_w_q, A_w_uk, A_w_uv, A_w_o,
      B_wqkv, B_wo.reshape(HB, DH, M), gate_w.reshape(1, M))
    return out.reshape(1, S, M)
```

```python
import functools
import jax
import jax.numpy as jnp
from jax import lax
import jax.experimental.pallas as pl
import jax.experimental.pallas.tpu as pltpu

CFG = dict(wstart=2, tf32=0, rlpos=2, rot=0, bq=128, ck=256, cn=512, pr=2048, pre=1, post=2, rb=256, rs=32, seg="xlu")

LOG2E = 1.4426950408889634
NT = (((1,), (1,)), ((), ()))
NN = (((1,), (0,)), ((), ()))
LANES = 128
f32, bf16 = jnp.float32, jnp.bfloat16


def _dot(a, b, dims=NN):
    return lax.dot_general(a, b, dims, preferred_element_type=jnp.float32)


def _kernel(x_hbm, c_hbm, wq_hbm, wuk_hbm, wuv_hbm, wo_hbm, bw_hbm, bwo_hbm, gw_hbm,
            out_hbm,
            x_v, c_v, wq_raw, wuk_raw, wuv_raw, wq_v, wuk_v, wuv_v, wo_v, bw_raw, bwt_v, bw_v, bwo_raw, bwo_v, gw_v,
            acc_v, out_v, g_v, q_s, k_s, v_s, q_n, k_n, v_n, s_s, bq_s, bk_s, bv_s, bp_s, sems, osems, xsems,
            *, S, M, Dc, H, D, HB, DH, W, DIL):
    NEG = -1e9 * LOG2E
    NJ = M // LANES
    PAD = W * DIL

    RB, RS = CFG["rb"], CFG["rs"]
    NCH = S // RB
    MQ, MC = M // NCH, Dc // NCH

    def cp(src, dst, i):
        return pltpu.make_async_copy(src, dst, sems.at[i])

    def x_copy(i):
        return pltpu.make_async_copy(x_hbm.at[pl.ds(i * RB, RB), :], x_v.at[pl.ds(i * RB, RB), :], xsems.at[0, i])

    def w_copies(i):
        return [pltpu.make_async_copy(src.at[pl.ds(i * n * H, n * H)], dst.at[pl.ds(i * n * H, n * H)], xsems.at[1 + k, i])
                for k, (src, dst, n) in enumerate(((wq_hbm, wq_raw, MQ), (wuk_hbm, wuk_raw, MC), (wuv_hbm, wuv_raw, MC)))]

    bw_cp = [cp(bw_hbm.at[:, pl.ds(t * M, M)], bw_raw.at[:, pl.ds(t * M, M)], t) for t in range(3)]
    copies = dict(gw=cp(gw_hbm, gw_v, 3), bwo=cp(bwo_hbm, bwo_raw, 4), c=cp(c_hbm, c_v, 5), wo=cp(wo_hbm, wo_v, 6))
    bw_cp[0].start()
    x_copy(0).start()
    copies["gw"].start()
    for i in range(1, NCH):
        x_copy(i).start()
    bw_cp[1].start()
    bw_cp[2].start()
    copies["bwo"].start()
    if CFG["wstart"] == 0:
        for i in range(NCH):
            for c_ in w_copies(i):
                c_.start()
        copies["c"].start()
        copies["wo"].start()

    def perm_qkv(t):
        bw_cp[t].wait()
        for n0 in range(0, M, LANES):
            wt = bw_raw[:, t * M + n0:t * M + n0 + LANES]
            wt = wt.astype(f32).T.astype(bf16) if CFG["tf32"] else wt.T
            bwt_v[n0 // DH:n0 // DH + LANES // DH] = wt.reshape(LANES // DH, DH, M)
        for m0 in range(0, M, 256):
            w3 = jnp.swapaxes(bwt_v[:, :, m0:m0 + 256], 0, 1)
            bw_v[t * M:(t + 1) * M, m0:m0 + 256] = w3.reshape(M, 256)

    def perm_o():
        copies["bwo"].wait()
        for m0 in range(0, M, 256):
            w3 = jnp.swapaxes(bwo_raw[:, :, m0:m0 + 256], 0, 1)
            bwo_v[:, m0:m0 + 256] = w3.reshape(M, 256)

    with jax.named_scope("b_perm"):
        perm_qkv(0)
        bk_s[0:PAD, :] = jnp.zeros((PAD, M), f32)
        bv_s[0:PAD, :] = jnp.zeros((PAD, M), f32)
        copies["gw"].wait()

    sc_b = DH ** -0.5 * LOG2E

    def b_pre(ci, carry):
        r0 = pl.multiple_of(ci * RB, RB)
        x_copy(ci).wait()
        if CFG["wstart"] == 1:
            @pl.when(ci >= NCH // 2)
            def _():
                for c_ in w_copies(2 * ci - NCH) + w_copies(2 * ci - NCH + 1):
                    c_.start()
        xr = x_v[pl.ds(r0, RB), :]
        gw = gw_v[...].astype(f32)
        t = None
        for j in range(NJ):
            p = xr[:, j * LANES:(j + 1) * LANES].astype(f32) * gw[:, j * LANES:(j + 1) * LANES]
            t = p if t is None else t + p
        g_v[pl.ds(r0, RB), :] = jnp.broadcast_to(jax.nn.sigmoid(jnp.sum(t, axis=1, keepdims=True)), (RB, LANES))
        bq_s[pl.ds(r0, RB), :] = _dot(xr, bw_v[0:M, :], NT) * sc_b
        return carry

    def relayout(ci):
        for c_ in w_copies(ci):
            c_.wait()
        for j in range(H // 2):
            for raw, dst, n in ((wq_raw, wq_v, MQ), (wuk_raw, wuk_v, MC), (wuv_raw, wuv_v, MC)):
                m0 = pl.multiple_of(ci * n, n)
                view = raw.bitcast(jnp.uint32).at[pl.ds(m0 * (H // 2), n * (H // 2)), :]
                v = view[pl.ds(j, n, stride=H // 2), :]
                dst[2 * j, pl.ds(m0, n), :] = pltpu.bitcast(v << 16, f32).astype(bf16)
                dst[2 * j + 1, pl.ds(m0, n), :] = pltpu.bitcast(v & jnp.uint32(0xFFFF0000), f32).astype(bf16)

    def b_chunk(ci, carry):
        r0 = pl.multiple_of(ci * RB, RB)
        xr = x_v[pl.ds(r0, RB), :]
        if CFG["rlpos"] == 0:
            relayout(ci)
        bk_s[PAD:PAD + RB, :] = _dot(xr, bw_v[M:2 * M, :], NT)
        if CFG["rlpos"] == 1:
            relayout(ci)
        bv_s[PAD:PAD + RB, :] = _dot(xr, bw_v[2 * M:3 * M, :], NT)
        if CFG["seg"] == "mxu":
            ri = lax.broadcasted_iota(jnp.int32, (LANES, LANES), 0)
            cj = lax.broadcasted_iota(jnp.int32, (LANES, LANES), 1)
            E = jnp.where(ri % HB == cj % HB, 1.0, 0.0).astype(bf16)
        for s0 in range(0, RB, RS):
            lg = [None] * W
            for j in range(NJ):
                q = bq_s[pl.ds(r0 + s0, RS), j * LANES:(j + 1) * LANES]
                for w in range(W):
                    st = PAD + s0 - w * DIL
                    p = q * bk_s[st:st + RS, j * LANES:(j + 1) * LANES]
                    lg[w] = p if lg[w] is None else lg[w] + p
            for w in range(W):
                l = lg[w]
                if CFG["seg"] == "mxu":
                    hi = l.astype(bf16)
                    lo = (l - hi.astype(f32)).astype(bf16)
                    l = _dot(hi, E) + _dot(lo, E)
                else:
                    sh = LANES // 2
                    while sh >= HB:
                        l = l + pltpu.roll(l, sh, 1)
                        sh //= 2
                if s0 < w * DIL:
                    rows = lax.broadcasted_iota(jnp.int32, (RS, LANES), 0) + (s0 + r0)
                    l = jnp.where(rows >= w * DIL, l, NEG)
                lg[w] = l
            m = functools.reduce(jnp.maximum, lg)
            ps = [jnp.exp2(l - m) for l in lg]
            den = functools.reduce(lambda a, b: a + b, ps)
            inv = (1.0 - g_v[pl.ds(r0 + s0, RS), :]) / den
            for w in range(W):
                bp_s[w, s0:s0 + RS, :] = ps[w] * inv
        if CFG["rlpos"] == 2:
            relayout(ci)
        out = None
        for j in range(NJ):
            o = None
            for w in range(W):
                st = PAD - w * DIL
                pv = bp_s[w] * bv_s[st:st + RB, j * LANES:(j + 1) * LANES]
                o = pv if o is None else o + pv
            d = _dot(o.astype(bf16), bwo_v[j * LANES:(j + 1) * LANES, :])
            out = d if out is None else out + d
        acc_v[pl.ds(r0, RB), :] = out
        bk_s[0:PAD, :] = bk_s[RB:RB + PAD, :]
        bv_s[0:PAD, :] = bv_s[RB:RB + PAD, :]
        if CFG["rlpos"] == 3:
            relayout(ci)
        return carry

    with jax.named_scope("b_pre"):
        lax.fori_loop(0, NCH, b_pre, 0)
    with jax.named_scope("b_perm2"):
        if CFG["wstart"] == 2:
            for i in range(NCH):
                for c_ in w_copies(i):
                    c_.start()
        if CFG["wstart"] > 0:
            copies["c"].start()
            copies["wo"].start()
        perm_qkv(1)
        perm_qkv(2)
        perm_o()
    with jax.named_scope("b_main"):
        lax.fori_loop(0, S // RB, b_chunk, 0)

    with jax.named_scope("a_wait"):
        copies["c"].wait()
        copies["wo"].wait()

    BQ, CK, CN = CFG["bq"], CFG["ck"], CFG["cn"]
    T = LANES
    NA = BQ // T
    sc_a = D ** -0.5 * LOG2E

    def pieces(i):
        r0 = i * BQ
        ps = [(0, k0, min(k0 + CK, r0), False) for k0 in range(0, r0, CK)]
        ps += [(b, r0 + b * T, r0 + (b + 1) * T, True) for b in range(NA)]
        return ps

    PR = CFG["pr"]

    def proj_pieces(hn, qd, kd, vd):
        def pq(r):
            qd[r:r + PR, :] = (_dot(x_v[r:r + PR, :], wq_v[hn]) * sc_a).astype(bf16)
        def pk(r):
            kd[r:r + PR, :] = _dot(c_v[r:r + PR, :], wuk_v[hn]).astype(bf16)
        def pvv(r):
            vd[r:r + PR, :] = _dot(c_v[r:r + PR, :], wuv_v[hn]).astype(bf16)
        qk_, v_ = [], []
        for r in range(0, S, PR):
            qk_.append([functools.partial(pk, r), functools.partial(pq, r)])
            v_.append([functools.partial(pvv, r)])
        lag = min(CFG["post"], S // PR)
        out = []
        for n in range(len(qk_) + lag):
            if n < len(qk_):
                out += qk_[n]
            if n >= lag:
                out += v_[n - lag]
        return out

    def copy_pieces(pairs):
        def cpy(src, dst, r):
            dst[r:r + 256, :] = src[r:r + 256, :]
        return [functools.partial(cpy, a_, b_, r) for r in range(0, S, 256) for a_, b_ in pairs]

    def a_head(h, last):
        row = lax.broadcasted_iota(jnp.int32, (T, T), 0)
        col = lax.broadcasted_iota(jnp.int32, (T, T), 1)
        cmask = col <= row
        st = {}

        def acc(lst, a, v, op):
            lst[a] = v if lst[a] is None else op(lst[a], v)

        def qk(i, pc):
            a0, k0, k1, diag = pc
            d = st.setdefault(i, dict(mr=[None] * NA, m=[None] * NA, l=[None] * NA, o=[None] * NA))
            r0 = i * BQ
            sc = _dot(q_s[r0 + a0 * T:r0 + BQ, :], k_s[k0:k1, :], NT)
            for a in range(a0, NA):
                sa = sc[(a - a0) * T:(a - a0 + 1) * T]
                if diag and a == a0:
                    sa = jnp.where(cmask, sa, NEG)
                s_s[i % 2, a * T:(a + 1) * T, k0:k1] = sa
                acc(d["mr"], a, functools.reduce(jnp.maximum, [sa[:, t:t + T] for t in range(0, k1 - k0, T)]),
                    jnp.maximum)

        def fin_m(i):
            d = st[i]
            for a in range(NA):
                d["m"][a] = jnp.max(d["mr"][a], axis=1, keepdims=True)

        def pv(i, pc):
            a0, k0, k1, diag = pc
            d = st[i]
            ps = []
            for a in range(a0, NA):
                p = jnp.exp2(s_s[i % 2, a * T:(a + 1) * T, k0:k1] - d["m"][a])
                acc(d["l"], a, functools.reduce(lambda u, v: u + v, [p[:, t:t + T] for t in range(0, k1 - k0, T)]),
                    lambda u, v: u + v)
                ps.append(p.astype(bf16))
            o = _dot(ps[0] if len(ps) == 1 else jnp.concatenate(ps, axis=0), v_s[k0:k1, :])
            for a in range(a0, NA):
                acc(d["o"], a, o[(a - a0) * T:(a - a0 + 1) * T], lambda u, v: u + v)

        def fin_o(i):
            d = st[i]
            r0 = i * BQ
            ctx = []
            for a in range(NA):
                l = jnp.sum(d["l"][a], axis=1, keepdims=True)
                ctx.append((d["o"][a] * (g_v[r0 + a * T:r0 + (a + 1) * T, :] / l)).astype(bf16))
            d["ctx"] = ctx[0] if NA == 1 else jnp.concatenate(ctx, axis=0)

        def outp(i, n0):
            r0 = i * BQ
            upd = acc_v[r0:r0 + BQ, n0:n0 + CN] + _dot(st[i]["ctx"], wo_v[h, :, n0:n0 + CN])
            if not last:
                acc_v[r0:r0 + BQ, n0:n0 + CN] = upd
            else:
                out_v[r0:r0 + BQ, n0:n0 + CN] = upd.astype(out_v.dtype)
                if n0 + CN == M:
                    out_copy(i).start()

        def interleave(*streams):
            streams = [s_ for s_ in streams if s_]
            n = max(len(s_) for s_ in streams)
            pos = [0] * len(streams)
            for t in range(n):
                for j, s_ in enumerate(streams):
                    want = ((t + 1) * len(s_) + n - 1) // n
                    while pos[j] < want:
                        s_[pos[j]]()
                        pos[j] += 1

        nq = S // BQ
        rot = CFG["rot"]
        if not rot:
            for f_ in proj_pieces(h, q_s, k_s, v_s):
                f_()
        nxt = [] if (last or not rot) else proj_pieces(h + 1, q_n, k_n, v_n)
        wts = [len(pieces(i)) * 2 + 2 for i in range(nq)]
        cum, tot, lo = 0, sum(wts), 0
        head_n = CFG["pre"]
        for pc in pieces(0):
            qk(0, pc)
        for f_ in nxt[:head_n]:
            f_()
        lo = head_n
        for i in range(nq):
            fin_m(i)
            cum += wts[i]
            hi = max(lo, min(len(nxt), head_n + ((len(nxt) - head_n - CFG["post"]) * cum + tot - 1) // tot))
            s_qk = [functools.partial(qk, i + 1, pc) for pc in pieces(i + 1)] if i + 1 < nq else []
            s_pv = [functools.partial(pv, i, pc) for pc in pieces(i)]
            s_o = [functools.partial(outp, i - 1, n0) for n0 in range(0, M, CN)] if i > 0 else []
            s_c = copy_pieces([(q_n, q_s), (k_n, k_s)]) if (i == nq - 1 and not last and rot) else []
            if s_c:
                for f_ in nxt[lo:hi]:
                    f_()
                lo = hi
            interleave(s_qk, s_pv, s_o, nxt[lo:hi], s_c)
            lo = hi
            fin_o(i)
        interleave([functools.partial(outp, nq - 1, n0) for n0 in range(0, M, CN)], nxt[lo:])
        if rot and not last:
            for f_ in copy_pieces([(v_n, v_s)]):
                f_()

    nq_ = S // BQ

    def out_copy(i):
        return pltpu.make_async_copy(out_v.at[pl.ds(i * BQ, BQ), :], out_hbm.at[pl.ds(i * BQ, BQ), :], osems.at[i])

    with jax.named_scope("a_first"):
        for f_ in (proj_pieces(0, q_s, k_s, v_s) if CFG["rot"] else []):
            f_()
    with jax.named_scope("a_main"):
        lax.fori_loop(0, H - 1, lambda h, c_: (a_head(h, False), c_)[1], 0)
    with jax.named_scope("a_last"):
        a_head(H - 1, True)
        for i in range(nq_):
            out_copy(i).wait()


@jax.jit
def pallas_gated_mix__compressed_kv_cla__sliding_local_dilated__prompt_kernel(
A_x: jax.Array,
    A_c_kv: jax.Array,
    A_w_q: jax.Array,
    A_w_uk: jax.Array,
    A_w_uv: jax.Array,
    A_w_o: jax.Array,
    B_x: jax.Array,
    B_wqkv: jax.Array,
    B_wo: jax.Array,
    gate_w: jax.Array,
):
    del B_x
    _, S, M = A_x.shape
    Dc = A_c_kv.shape[2]
    _, H, D = A_w_q.shape
    HB, W, DIL = 32, 8, 2
    DH = M // HB
    PAD = W * DIL
    RB = CFG["rb"]
    dt = A_x.dtype
    hbm = pl.BlockSpec(memory_space=pltpu.MemorySpace.HBM)
    V = pltpu.VMEM
    kern = functools.partial(_kernel, S=S, M=M, Dc=Dc, H=H, D=D, HB=HB, DH=DH, W=W, DIL=DIL)
    out = pl.pallas_call(
        kern,
        in_specs=[hbm] * 9,
        out_specs=hbm,
        out_shape=jax.ShapeDtypeStruct((S, M), dt),
        scratch_shapes=[
            V((S, M), dt), V((S, Dc), dt),
            V((M * H, D), dt), V((Dc * H, D), dt), V((Dc * H, D), dt),
            V((H, M, D), dt), V((H, Dc, D), dt), V((H, Dc, D), dt), V((H, D, M), dt),
            V((M, 3 * M), dt), V((HB, DH, M), dt), V((3 * M, M), dt),
            V((HB, DH, M), dt), V((M, M), dt), V((1, M), dt),
            V((S, M), f32), V((S, M), dt), V((S, LANES), f32),
            V((S, D), dt), V((S, D), dt), V((S, D), dt), V((S, D), dt), V((S, D), dt), V((S, D), dt), V((2, CFG["bq"], S), f32),
            V((S, M), f32), V((RB + PAD, M), f32), V((RB + PAD, M), f32), V((W, RB, LANES), f32),
            pltpu.SemaphoreType.DMA((10,)), pltpu.SemaphoreType.DMA((S // CFG["bq"],)),
            pltpu.SemaphoreType.DMA((4, S // RB)),
        ],
        compiler_params=pltpu.CompilerParams(vmem_limit_bytes=110 * 1024 * 1024),
    )(A_x.reshape(S, M), A_c_kv.reshape(S, Dc), A_w_q.reshape(M * H, D), A_w_uk.reshape(Dc * H, D),
      A_w_uv.reshape(Dc * H, D), A_w_o,
      B_wqkv, B_wo.reshape(HB, DH, M), gate_w.reshape(1, M))
    return out.reshape(1, S, M)
```

```python
import functools
import jax
import jax.numpy as jnp
from jax import lax
import jax.experimental.pallas as pl
import jax.experimental.pallas.tpu as pltpu

CFG = dict(ph=(4, -10, -1), wstart=2, tf32=0, rlpos=2, rot=0, bq=128, ck=128, cn=512, pr=512, pre=1, post=2, rb=256, rs=32, seg="xlu")

LOG2E = 1.4426950408889634
NT = (((1,), (1,)), ((), ()))
NN = (((1,), (0,)), ((), ()))
LANES = 128
f32, bf16 = jnp.float32, jnp.bfloat16


def _dot(a, b, dims=NN):
    return lax.dot_general(a, b, dims, preferred_element_type=jnp.float32)


def _kernel(x_hbm, c_hbm, wq_hbm, wuk_hbm, wuv_hbm, wo_hbm, bw_hbm, bwo_hbm, gw_hbm,
            out_hbm,
            x_v, c_v, wq_raw, wuk_raw, wuv_raw, wq_v, wuk_v, wuv_v, wo_v, bw_raw, bwt_v, bw_v, bwo_raw, bwo_v, gw_v,
            acc_v, out_v, g_v, q_s, k_s, v_s, ux_v, uc_v, s_s, bq_s, bk_s, bv_s, bp_s, sems, osems, xsems,
            *, S, M, Dc, H, D, HB, DH, W, DIL):
    NEG = -1e9 * LOG2E
    NJ = M // LANES
    PAD = W * DIL

    RB, RS = CFG["rb"], CFG["rs"]
    NCH = S // RB
    MQ, MC = M // NCH, Dc // NCH

    def cp(src, dst, i):
        return pltpu.make_async_copy(src, dst, sems.at[i])

    def x_copy(i):
        return pltpu.make_async_copy(x_hbm.at[pl.ds(i * RB, RB), :], x_v.at[pl.ds(i * RB, RB), :], xsems.at[0, i])

    def w_copies(i):
        return [pltpu.make_async_copy(src.at[pl.ds(i * n * H, n * H)], dst.at[pl.ds(i * n * H, n * H)], xsems.at[1 + k, i])
                for k, (src, dst, n) in enumerate(((wq_hbm, wq_raw, MQ), (wuk_hbm, wuk_raw, MC), (wuv_hbm, wuv_raw, MC)))]

    bw_cp = [cp(bw_hbm.at[:, pl.ds(t * M, M)], bw_raw.at[:, pl.ds(t * M, M)], t) for t in range(3)]
    copies = dict(gw=cp(gw_hbm, gw_v, 3), bwo=cp(bwo_hbm, bwo_raw, 4), c=cp(c_hbm, c_v, 5), wo=cp(wo_hbm, wo_v, 6))
    bw_cp[0].start()
    x_copy(0).start()
    copies["gw"].start()
    for i in range(1, NCH):
        x_copy(i).start()
    bw_cp[1].start()
    bw_cp[2].start()
    copies["bwo"].start()
    if CFG["wstart"] == 0:
        for i in range(NCH):
            for c_ in w_copies(i):
                c_.start()
        copies["c"].start()
        copies["wo"].start()

    def perm_qkv(t):
        bw_cp[t].wait()
        for n0 in range(0, M, LANES):
            wt = bw_raw[:, t * M + n0:t * M + n0 + LANES]
            wt = wt.astype(f32).T.astype(bf16) if CFG["tf32"] else wt.T
            bwt_v[n0 // DH:n0 // DH + LANES // DH] = wt.reshape(LANES // DH, DH, M)
        for m0 in range(0, M, 256):
            w3 = jnp.swapaxes(bwt_v[:, :, m0:m0 + 256], 0, 1)
            bw_v[t * M:(t + 1) * M, m0:m0 + 256] = w3.reshape(M, 256)

    def perm_o():
        copies["bwo"].wait()
        for m0 in range(0, M, 256):
            w3 = jnp.swapaxes(bwo_raw[:, :, m0:m0 + 256], 0, 1)
            bwo_v[:, m0:m0 + 256] = w3.reshape(M, 256)

    with jax.named_scope("b_perm"):
        perm_qkv(0)
        bk_s[0:PAD, :] = jnp.zeros((PAD, M), f32)
        bv_s[0:PAD, :] = jnp.zeros((PAD, M), f32)
        copies["gw"].wait()

    sc_b = DH ** -0.5 * LOG2E

    def b_pre(ci, carry):
        r0 = pl.multiple_of(ci * RB, RB)
        x_copy(ci).wait()
        if CFG["wstart"] == 1:
            @pl.when(ci >= NCH // 2)
            def _():
                for c_ in w_copies(2 * ci - NCH) + w_copies(2 * ci - NCH + 1):
                    c_.start()
        xr = x_v[pl.ds(r0, RB), :]
        gw = gw_v[...].astype(f32)
        t = None
        for j in range(NJ):
            p = xr[:, j * LANES:(j + 1) * LANES].astype(f32) * gw[:, j * LANES:(j + 1) * LANES]
            t = p if t is None else t + p
        g_v[pl.ds(r0, RB), :] = jnp.broadcast_to(jax.nn.sigmoid(jnp.sum(t, axis=1, keepdims=True)), (RB, LANES))
        bq_s[pl.ds(r0, RB), :] = _dot(xr, bw_v[0:M, :], NT) * sc_b
        return carry

    def relayout(ci):
        for c_ in w_copies(ci):
            c_.wait()
        for j in range(H // 2):
            for raw, dst, n in ((wq_raw, wq_v, MQ), (wuk_raw, wuk_v, MC), (wuv_raw, wuv_v, MC)):
                m0 = pl.multiple_of(ci * n, n)
                view = raw.bitcast(jnp.uint32).at[pl.ds(m0 * (H // 2), n * (H // 2)), :]
                v = view[pl.ds(j, n, stride=H // 2), :]
                dst[2 * j, pl.ds(m0, n), :] = pltpu.bitcast(v << 16, f32).astype(bf16)
                dst[2 * j + 1, pl.ds(m0, n), :] = pltpu.bitcast(v & jnp.uint32(0xFFFF0000), f32).astype(bf16)

    def b_chunk(ci, carry):
        r0 = pl.multiple_of(ci * RB, RB)
        xr = x_v[pl.ds(r0, RB), :]
        if CFG["rlpos"] == 0:
            relayout(ci)
        bk_s[PAD:PAD + RB, :] = _dot(xr, bw_v[M:2 * M, :], NT)
        if CFG["rlpos"] == 1:
            relayout(ci)
        bv_s[PAD:PAD + RB, :] = _dot(xr, bw_v[2 * M:3 * M, :], NT)
        if CFG["seg"] == "mxu":
            ri = lax.broadcasted_iota(jnp.int32, (LANES, LANES), 0)
            cj = lax.broadcasted_iota(jnp.int32, (LANES, LANES), 1)
            E = jnp.where(ri % HB == cj % HB, 1.0, 0.0).astype(bf16)
        for s0 in range(0, RB, RS):
            lg = [None] * W
            for j in range(NJ):
                q = bq_s[pl.ds(r0 + s0, RS), j * LANES:(j + 1) * LANES]
                for w in range(W):
                    st = PAD + s0 - w * DIL
                    p = q * bk_s[st:st + RS, j * LANES:(j + 1) * LANES]
                    lg[w] = p if lg[w] is None else lg[w] + p
            for w in range(W):
                l = lg[w]
                if CFG["seg"] == "mxu":
                    hi = l.astype(bf16)
                    lo = (l - hi.astype(f32)).astype(bf16)
                    l = _dot(hi, E) + _dot(lo, E)
                else:
                    sh = LANES // 2
                    while sh >= HB:
                        l = l + pltpu.roll(l, sh, 1)
                        sh //= 2
                if s0 < w * DIL:
                    rows = lax.broadcasted_iota(jnp.int32, (RS, LANES), 0) + (s0 + r0)
                    l = jnp.where(rows >= w * DIL, l, NEG)
                lg[w] = l
            m = functools.reduce(jnp.maximum, lg)
            ps = [jnp.exp2(l - m) for l in lg]
            den = functools.reduce(lambda a, b: a + b, ps)
            inv = (1.0 - g_v[pl.ds(r0 + s0, RS), :]) / den
            for w in range(W):
                bp_s[w, s0:s0 + RS, :] = ps[w] * inv
        if CFG["rlpos"] == 2:
            relayout(ci)
        out = None
        for j in range(NJ):
            o = None
            for w in range(W):
                st = PAD - w * DIL
                pv = bp_s[w] * bv_s[st:st + RB, j * LANES:(j + 1) * LANES]
                o = pv if o is None else o + pv
            d = _dot(o.astype(bf16), bwo_v[j * LANES:(j + 1) * LANES, :])
            out = d if out is None else out + d
        acc_v[pl.ds(r0, RB), :] = out
        bk_s[0:PAD, :] = bk_s[RB:RB + PAD, :]
        bv_s[0:PAD, :] = bv_s[RB:RB + PAD, :]
        if CFG["rlpos"] == 3:
            relayout(ci)
        return carry

    with jax.named_scope("b_pre"):
        lax.fori_loop(0, NCH, b_pre, 0)
    with jax.named_scope("b_perm2"):
        if CFG["wstart"] == 2:
            for i in range(NCH):
                for c_ in w_copies(i):
                    c_.start()
        if CFG["wstart"] > 0:
            copies["c"].start()
            copies["wo"].start()
        perm_qkv(1)
        perm_qkv(2)
        perm_o()
    with jax.named_scope("b_main"):
        lax.fori_loop(0, S // RB, b_chunk, 0)

    BQ, CK, CN = CFG["bq"], CFG["ck"], CFG["cn"]
    T = LANES
    NA = BQ // T
    sc_a = D ** -0.5 * LOG2E

    def pieces(i):
        r0 = i * BQ
        ps = [(0, k0, min(k0 + CK, r0), False) for k0 in range(0, r0, CK)]
        ps += [(b, r0 + b * T, r0 + (b + 1) * T, True) for b in range(NA)]
        return ps

    PR = CFG["pr"]
    SH = S // 2

    def add(a, b):
        return (a.astype(f32) + b.astype(f32)).astype(bf16)

    def sub(a, b):
        return (a.astype(f32) - b.astype(f32)).astype(bf16)

    def strassen_lhs(src, u):
        kh = src.shape[1] // 2
        def body(i, carry):
            r = pl.multiple_of(i * 128, 128)
            top, bot = pl.ds(r, 128), pl.ds(SH + r, 128)
            a11, a12, a21, a22 = src[top, 0:kh], src[top, kh:2 * kh], src[bot, 0:kh], src[bot, kh:2 * kh]
            u[0, top, :] = add(a11, a22)
            u[1, top, :] = add(a21, a22)
            u[2, top, :] = add(a11, a12)
            u[3, top, :] = sub(a21, a11)
            u[4, top, :] = sub(a12, a22)
            return carry
        lax.fori_loop(0, SH // 128, body, 0)

    def proj_pair(p, src, u, w, dst, scale):
        kh = src.shape[1] // 2
        we, wo_ = w.at[2 * p], w.at[2 * p + 1]
        b11, b21, b12, b22 = we[0:kh, :], we[kh:2 * kh, :], wo_[0:kh, :], wo_[kh:2 * kh, :]
        t1, t3, t4, t6, t7 = add(b11, b22), sub(b12, b22), sub(b21, b11), add(b11, b12), add(b21, b22)
        for r in range(0, SH, PR):
            top, bot = slice(r, r + PR), slice(SH + r, SH + r + PR)
            m2 = _dot(u[1, top, :], b11)
            m5 = _dot(u[2, top, :], b22)
            m4 = _dot(src[bot, kh:2 * kh], t4)
            m3 = _dot(src[top, 0:kh], t3)
            m1 = _dot(u[0, top, :], t1)
            m7 = _dot(u[4, top, :], t7)
            m6 = _dot(u[3, top, :], t6)
            dst[0, bot, :] = ((m2 + m4) * scale).astype(bf16)
            dst[1, top, :] = ((m3 + m5) * scale).astype(bf16)
            dst[0, top, :] = ((m1 + m4 - m5 + m7) * scale).astype(bf16)
            dst[1, bot, :] = ((m1 - m2 + m3 + m6) * scale).astype(bf16)

    def a_pair(p, last):
        proj_pair(p, c_v, uc_v, wuk_v, k_s, 1.0)
        proj_pair(p, x_v, ux_v, wq_v, q_s, sc_a)
        proj_pair(p, c_v, uc_v, wuv_v, v_s, 1.0)
        a_head(2 * p, 0, False)
        a_head(2 * p + 1, 1, last)

    def a_head(h, e, last):
        row = lax.broadcasted_iota(jnp.int32, (T, T), 0)
        col = lax.broadcasted_iota(jnp.int32, (T, T), 1)
        cmask = col <= row
        st = {}

        def acc(lst, a, v, op):
            lst[a] = v if lst[a] is None else op(lst[a], v)

        def qk(i, pc):
            a0, k0, k1, diag = pc
            d = st.setdefault(i, dict(mr=[None] * NA, m=[None] * NA, l=[None] * NA, o=[None] * NA))
            r0 = i * BQ
            sc = _dot(q_s[e, r0 + a0 * T:r0 + BQ, :], k_s[e, k0:k1, :], NT)
            for a in range(a0, NA):
                sa = sc[(a - a0) * T:(a - a0 + 1) * T]
                if diag and a == a0:
                    sa = jnp.where(cmask, sa, NEG)
                s_s[i % 2, a * T:(a + 1) * T, k0:k1] = sa
                acc(d["mr"], a, functools.reduce(jnp.maximum, [sa[:, t:t + T] for t in range(0, k1 - k0, T)]),
                    jnp.maximum)

        def fin_m(i):
            d = st[i]
            for a in range(NA):
                d["m"][a] = jnp.max(d["mr"][a], axis=1, keepdims=True)

        def pv(i, pc):
            a0, k0, k1, diag = pc
            d = st[i]
            ps = []
            for a in range(a0, NA):
                p = jnp.exp2(s_s[i % 2, a * T:(a + 1) * T, k0:k1] - d["m"][a])
                acc(d["l"], a, functools.reduce(lambda u, v: u + v, [p[:, t:t + T] for t in range(0, k1 - k0, T)]),
                    lambda u, v: u + v)
                ps.append(p.astype(bf16))
            o = _dot(ps[0] if len(ps) == 1 else jnp.concatenate(ps, axis=0), v_s[e, k0:k1, :])
            for a in range(a0, NA):
                acc(d["o"], a, o[(a - a0) * T:(a - a0 + 1) * T], lambda u, v: u + v)

        def fin_o(i):
            d = st[i]
            r0 = i * BQ
            ctx = []
            for a in range(NA):
                l = jnp.sum(d["l"][a], axis=1, keepdims=True)
                ctx.append((d["o"][a] * (g_v[r0 + a * T:r0 + (a + 1) * T, :] / l)).astype(bf16))
            d["ctx"] = ctx[0] if NA == 1 else jnp.concatenate(ctx, axis=0)

        def outp(i, n0):
            r0 = i * BQ
            upd = acc_v[r0:r0 + BQ, n0:n0 + CN] + _dot(st[i]["ctx"], wo_v[h, :, n0:n0 + CN])
            if not last:
                acc_v[r0:r0 + BQ, n0:n0 + CN] = upd
            else:
                out_v[r0:r0 + BQ, n0:n0 + CN] = upd.astype(out_v.dtype)
                if n0 + CN == M:
                    out_copy(i).start()

        def interleave(*streams):
            streams = [s_ for s_ in streams if s_]
            n = max(len(s_) for s_ in streams)
            pos = [0] * len(streams)
            for t in range(n):
                for j, s_ in enumerate(streams):
                    want = (min(len(s_), ((t + 1) * len(s_) + (n - 1) * CFG["ph"][j] // 4) // n)
                            if t + 1 < n else len(s_))
                    while pos[j] < want:
                        s_[pos[j]]()
                        pos[j] += 1

        nq = S // BQ
        for pc in pieces(0):
            qk(0, pc)
        for i in range(nq):
            fin_m(i)
            s_qk = [functools.partial(qk, i + 1, pc) for pc in pieces(i + 1)] if i + 1 < nq else []
            s_pv = [functools.partial(pv, i, pc) for pc in pieces(i)]
            s_o = [functools.partial(outp, i - 1, n0) for n0 in range(0, M, CN)] if i > 0 else []
            interleave(s_qk, s_pv, s_o)
            fin_o(i)
        for n0 in range(0, M, CN):
            outp(nq - 1, n0)

    nq_ = S // BQ

    def out_copy(i):
        return pltpu.make_async_copy(out_v.at[pl.ds(i * BQ, BQ), :], out_hbm.at[pl.ds(i * BQ, BQ), :], osems.at[i])

    with jax.named_scope("a_pre"):
        copies["c"].wait()
        strassen_lhs(x_v, ux_v)
        strassen_lhs(c_v, uc_v)
        copies["wo"].wait()
    with jax.named_scope("a_main"):
        lax.fori_loop(0, H // 2 - 1, lambda p, c_: (a_pair(p, False), c_)[1], 0)
    with jax.named_scope("a_last"):
        a_pair(H // 2 - 1, True)
        for i in range(nq_):
            out_copy(i).wait()


@jax.jit
def pallas_gated_mix__compressed_kv_cla__sliding_local_dilated__prompt_kernel(
A_x: jax.Array,
    A_c_kv: jax.Array,
    A_w_q: jax.Array,
    A_w_uk: jax.Array,
    A_w_uv: jax.Array,
    A_w_o: jax.Array,
    B_x: jax.Array,
    B_wqkv: jax.Array,
    B_wo: jax.Array,
    gate_w: jax.Array,
):
    del B_x
    _, S, M = A_x.shape
    Dc = A_c_kv.shape[2]
    _, H, D = A_w_q.shape
    HB, W, DIL = 32, 8, 2
    DH = M // HB
    PAD = W * DIL
    RB = CFG["rb"]
    dt = A_x.dtype
    hbm = pl.BlockSpec(memory_space=pltpu.MemorySpace.HBM)
    V = pltpu.VMEM
    kern = functools.partial(_kernel, S=S, M=M, Dc=Dc, H=H, D=D, HB=HB, DH=DH, W=W, DIL=DIL)
    out = pl.pallas_call(
        kern,
        in_specs=[hbm] * 9,
        out_specs=hbm,
        out_shape=jax.ShapeDtypeStruct((S, M), dt),
        scratch_shapes=[
            V((S, M), dt), V((S, Dc), dt),
            V((M * H, D), dt), V((Dc * H, D), dt), V((Dc * H, D), dt),
            V((H, M, D), dt), V((H, Dc, D), dt), V((H, Dc, D), dt), V((H, D, M), dt),
            V((M, 3 * M), dt), V((HB, DH, M), dt), V((3 * M, M), dt),
            V((HB, DH, M), dt), V((M, M), dt), V((1, M), dt),
            V((S, M), f32), V((S, M), dt), V((S, LANES), f32),
            V((2, S, D), dt), V((2, S, D), dt), V((2, S, D), dt),
            V((5, S // 2, M // 2), dt), V((5, S // 2, Dc // 2), dt), V((2, CFG["bq"], S), f32),
            V((S, M), f32), V((RB + PAD, M), f32), V((RB + PAD, M), f32), V((W, RB, LANES), f32),
            pltpu.SemaphoreType.DMA((10,)), pltpu.SemaphoreType.DMA((S // CFG["bq"],)),
            pltpu.SemaphoreType.DMA((4, S // RB)),
        ],
        compiler_params=pltpu.CompilerParams(vmem_limit_bytes=120 * 1024 * 1024),
    )(A_x.reshape(S, M), A_c_kv.reshape(S, Dc), A_w_q.reshape(M * H, D), A_w_uk.reshape(Dc * H, D),
      A_w_uv.reshape(Dc * H, D), A_w_o,
      B_wqkv, B_wo.reshape(HB, DH, M), gate_w.reshape(1, M))
    return out.reshape(1, S, M)
```
